```python
import jax
import jax.numpy as jnp

def _softmax(x, axis=-1):
    return jax.nn.softmax(x, axis=axis)
def _gelu(x):
    return jax.nn.gelu(x, approximate=True)
def _silu(x):
    return jax.nn.silu(x)
def _sigmoid(x):
    return jax.nn.sigmoid(x)
def _layernorm(x, axis=-1, eps=1e-5):
    m = jnp.mean(x, axis=axis, keepdims=True)
    v = jnp.var(x, axis=axis, keepdims=True)
    return (x - m) / jnp.sqrt(v + eps)
def _scatter_add(tgt, idx, src, axis=0):
    return tgt.at[idx].add(src)
def _segment_sum(src, seg, n):
    return jax.ops.segment_sum(src, seg, n)
class _Rng:
    def __init__(self, key):
        self._k = key
    def _next(self):
        self._k, sub = jax.random.split(self._k)
        return sub
    def normal(self, shape):
        return jax.random.normal(self._next(), shape, dtype=jnp.bfloat16)
    def randint(self, lo, hi, shape):
        return jax.random.randint(self._next(), shape, lo, hi, dtype=jnp.int32)
    def uniform(self, shape, lo=0.0, hi=1.0):
        return jax.random.uniform(self._next(), shape, jnp.bfloat16, lo, hi)
    def permutation(self, n):
        return jax.random.permutation(self._next(), n)


kernel_name = 'gated_mix__sliding_block_cached__glu_gated_swiglu__decode'

def setup_inputs():
    _rng = _Rng(jax.random.key(int.from_bytes(__import__("os").urandom(4), "little")))
    _w = (lambda a: (lambda t: t.astype(jnp.bfloat16) if jnp.issubdtype(t.dtype, jnp.floating) else t)(jnp.asarray(a)))
    def _A_setup():
        B, Sq, D = 1, 1, 640
        Hq, Hkv, Sk, Dh = 32, 32, 32768, 192
        assert Hq % Hkv == 0, (Hq, Hkv)
        return {
            "x": _w((lambda *s: _rng.normal(s) * 0.05)(B, Sq, D)),
            "k_cache": _w((lambda *s: _rng.normal(s) * 0.05)(B, Hkv, Sk, Dh)),
            "v_cache": _w((lambda *s: _rng.normal(s) * 0.05)(B, Hkv, Sk, Dh)),
            "wq": _w((lambda *s: _rng.normal(s) * 0.05)(D, Hq * Dh) * (D ** -0.5)),
            "wo": _w((lambda *s: _rng.normal(s) * 0.05)(Hq * Dh, D) * ((Hq * Dh) ** -0.5)),
        }
    _A_in = _A_setup()

    def _B_setup():
        B, S, D, F = 1, 1, 640, 1536
        return {
            "x": _w((lambda *s: _rng.normal(s) * 0.05)(B, S, D)),
            "w1": _w((lambda *s: _rng.normal(s) * 0.05)(D, F) * (2.0 / D) ** 0.5),
            "w3": _w((lambda *s: _rng.normal(s) * 0.05)(D, F) * (2.0 / D) ** 0.5),
            "w2": _w((lambda *s: _rng.normal(s) * 0.05)(F, D) * (2.0 / F) ** 0.5),
        }
    _B_in = _B_setup()

    return {
        "A_x": _A_in["x"],
        "A_k_cache": _A_in["k_cache"],
        "A_v_cache": _A_in["v_cache"],
        "A_wq": _A_in["wq"],
        "A_wo": _A_in["wo"],
        "B_x": _B_in["x"],
        "B_w1": _B_in["w1"],
        "B_w3": _B_in["w3"],
        "B_w2": _B_in["w2"],
        "gate_w": _w((lambda *s: _rng.normal(s) * 0.05)(640)),
    }

def reference(A_x, A_k_cache, A_v_cache, A_wq, A_wo, B_x, B_w1, B_w3, B_w2, gate_w):
    def _A_ref(x, k_cache, v_cache, wq, wo):
        B, Sq, D = x.shape
        Hq, Dh = 32, 192
        Hkv, Sk = k_cache.shape[1], k_cache.shape[2]
        W = min(4096, max(256, Sk // 4))
        rep = Hq // Hkv
        q = (lambda x, *d: x.transpose(*d))((x @ wq).reshape(B, Sq, Hq, Dh), 0, 2, 1, 3)
        k = jnp.repeat(k_cache[:, :, Sk - W:, :], rep, axis=1)
        v = jnp.repeat(v_cache[:, :, Sk - W:, :], rep, axis=1)
        scores = jnp.einsum("bhqd,bhkd->bhqk", q, k) * (Dh ** -0.5)
        p = _softmax(scores, axis=-1)
        o = jnp.einsum("bhqk,bhkd->bhqd", p, v)
        return (lambda x, *d: x.transpose(*d))(o, 0, 2, 1, 3).reshape(B, Sq, Hq * Dh) @ wo

    def _B_ref(x, w1, w3, w2):
        gate = jnp.einsum("bsd,df->bsf", x, w1)
        up = jnp.einsum("bsd,df->bsf", x, w3)
        h = _silu(gate) * up
        out = jnp.einsum("bsf,fd->bsd", h, w2)
        return out

    x = A_x
    g = _sigmoid((x * gate_w).sum(-1, keepdims=True))
    a = _A_ref(x, A_k_cache, A_v_cache, A_wq, A_wo)
    b = _B_ref(x, B_w1, B_w3, B_w2)
    return g * a + (1 - g) * b
```

```python
import functools
import jax
import jax.numpy as jnp
import numpy as np
import jax.experimental.pallas as pl
import jax.experimental.pallas.tpu as pltpu

H, DH, D, F = 32, 192, 640, 1536
M = 8
CW = 128
f32, bf16 = jnp.float32, jnp.bfloat16


def _kernel(x_hbm, k_hbm, v_hbm, wq_hbm, wo_hbm, w1_hbm, w3_hbm, w2_hbm, gw_hbm, o_ref,
            x_v, gw_v, wq_v, wo_v, w1_v, w3_v, w2_v, kbuf, vbuf, q_scr, s_scr, h_scr, b_scr,
            sems, sem_o, sem_s, *, SK, W, WQ, W13, G, SPLIT, WOPOS):
    NC = W // CW
    NO = D // 128
    R = 2 * NC
    GW = G * CW

    def par(h):
        return h % 2 if isinstance(h, int) else h & 1

    def k_copy(h, c):
        return pltpu.make_async_copy(k_hbm.at[0, h, :, pl.ds(SK - W + c * CW, CW)],
                                     kbuf.at[par(h), :, pl.ds(c * CW, CW)], sems.at[2 * c])

    def v_copy(h, c):
        return pltpu.make_async_copy(v_hbm.at[0, h, :, pl.ds(SK - W + c * CW, CW)],
                                     vbuf.at[par(h), :, pl.ds(c * CW, CW)], sems.at[2 * c + 1])

    def o_copy(h, i):
        r = pl.multiple_of(h * DH, 64)
        return pltpu.make_async_copy(wo_hbm.at[pl.ds(r, DH), pl.ds(i * 128, 128)],
                                     wo_v.at[par(h), :, pl.ds(i * 128, 128)], sem_o.at[i])

    blocks = []
    r13, c13 = W13
    for c in range(F // c13):
        for name, (src, dst) in (('g', (w1_hbm, w1_v)), ('u', (w3_hbm, w3_v))):
            blocks.append((name, c * c13, c13, [(src, dst, r * r13, r13, c * c13, c13) for r in range(D // r13)]))
    for c in range(D // 128):
        blocks.append(('b', c * 128, 128, [(w2_hbm, w2_v, r * DH, DH, c * 128, 128) for r in range(F // DH)]))
    rq, cq = WQ
    for c in range(H * DH // cq):
        blocks.append(('q', c * cq, cq, [(wq_hbm, wq_v, r * rq, rq, c * cq, cq) for r in range(D // rq)]))
    pro = [ch for b in blocks for ch in b[3]]
    P = len(pro)

    def t0_copy(j):
        if j < P:
            src, dst, r0, nr, c0, ncol = pro[j]
            return pltpu.make_async_copy(src.at[pl.ds(r0, nr), pl.ds(c0, ncol)], dst.at[pl.ds(r0, nr), pl.ds(c0, ncol)],
                                         sems.at[(j - P) % R])
        i = j - P
        return k_copy(0, i // 2) if i % 2 == 0 else v_copy(0, i // 2)

    def pri(j):
        return (j - P) % 2

    x_copy = pltpu.make_async_copy(x_hbm.at[0], x_v, sem_s.at[0])
    gw_copy = pltpu.make_async_copy(gw_hbm, gw_v, sem_s.at[1])
    x_copy.start()
    gw_copy.start()
    for j in range(R):
        t0_copy(j).start(priority=pri(j))
    x_copy.wait()
    gw_copy.wait()
    xb = jnp.broadcast_to(x_v[...], (M, D))
    xg = x_v[...].astype(f32) * gw_v[...].astype(f32).reshape(1, D)
    g = jax.nn.sigmoid(jnp.sum(xg, axis=-1, keepdims=True))

    j = 0
    gate = None
    for name, c0, ncol, chunks in blocks:
        for _ in chunks:
            t0_copy(j).wait()
            t0_copy(j + R).start(priority=pri(j + R))
            j += 1
        dst = chunks[0][1]
        if name == 'b':
            b_scr[:, pl.ds(c0, ncol)] = jnp.dot(h_scr[...], dst[:, pl.ds(c0, ncol)], preferred_element_type=f32)
        else:
            d = jnp.dot(xb, dst[:, pl.ds(c0, ncol)], preferred_element_type=f32)
            if name == 'q':
                qb = d.astype(bf16)
                for t in range(ncol // DH):
                    q_scr[c0 // DH + t] = qb[:, t * DH:(t + 1) * DH]
            elif name == 'g':
                gate = d
            else:
                h_scr[:, pl.ds(c0, ncol)] = (gate * jax.nn.sigmoid(gate) * d).astype(bf16)

    scale = DH ** -0.5
    wo_at = {c: i for i, c in enumerate(WOPOS)}

    def iteration(h, m_vec, out_acc, do_k, start_k, do_v, start_v, first_wo=False):
        ph, ph1 = par(h), par(h + 1)
        if do_v:
            m = jnp.max(m_vec, axis=-1, keepdims=True)
            l_vec = jnp.zeros((M, CW), f32)
            o_acc = jnp.zeros((M, DH), f32)
        m_new = jnp.full((M, CW), -jnp.inf, f32)
        if do_k:
            qh = q_scr[h + 1]

        def qk(gi):
            s = jnp.dot(qh, kbuf[ph1, :, pl.ds(gi * GW, GW)], preferred_element_type=f32) * scale
            s_scr[ph1, :, pl.ds(gi * GW, GW)] = s
            mm = m_new
            for t in range(G):
                mm = jnp.maximum(mm, s[:, t * CW:(t + 1) * CW])
            return mm

        def pv(gi):
            p = jnp.exp(s_scr[ph, :, pl.ds(gi * GW, GW)] - m)
            ll = l_vec
            for t in range(G):
                ll = ll + p[:, t * CW:(t + 1) * CW]
            oo = o_acc + jax.lax.dot_general(p.astype(bf16), vbuf[ph, :, pl.ds(gi * GW, GW)], (((1,), (1,)), ((), ())),
                                             preferred_element_type=f32)
            return ll, oo

        for gi in range(NC // G):
            for c in range(gi * G, (gi + 1) * G):
                if do_k:
                    k_copy(h + 1, c).wait()
                    if start_k:
                        k_copy(h + 2, c).start(priority=0)
                    if first_wo and c in wo_at:
                        o_copy(0, wo_at[c]).start(priority=1)
                if do_v:
                    v_copy(h, c).wait()
                    if start_v:
                        v_copy(h + 1, c).start(priority=1)
                    if c in wo_at:
                        o_copy(h, wo_at[c]).wait()
                        if start_v:
                            o_copy(h + 1, wo_at[c]).start(priority=wo_at[c] % 2)
                if SPLIT and do_k and do_v and c - gi * G == G // 2 - 1 and gi > 0:
                    pass
            if do_k:
                m_new = qk(gi)
            if do_v:
                l_vec, o_acc = pv(gi)
        if do_v:
            l = jnp.sum(l_vec, axis=-1, keepdims=True)
            o = (o_acc / l).astype(bf16)
            out_acc = out_acc + jnp.dot(o, wo_v[ph], preferred_element_type=f32)
        return m_new, out_acc

    out_acc = jnp.zeros((M, D), f32)
    m_vec, out_acc = iteration(-1, None, out_acc, True, True, False, False, first_wo=True)

    def loop(h, carry):
        return iteration(h, carry[0], carry[1], True, True, True, True)

    m_vec, out_acc = jax.lax.fori_loop(0, H - 2, loop, (m_vec, out_acc))
    m_vec, out_acc = iteration(H - 2, m_vec, out_acc, True, False, True, True)
    _, out_acc = iteration(H - 1, m_vec, out_acc, False, False, True, False)

    out = g * out_acc[0:1] + (1 - g) * b_scr[0:1, :]
    o_ref[0] = out.astype(o_ref.dtype)


def _make(WQ=(64, 384), W13=(64, 384), G=4, SPLIT=False, WOPOS=(2, 8, 14, 20, 26), **cp):
    def kernel(A_x, A_k_cache, A_v_cache, A_wq, A_wo, B_x, B_w1, B_w3, B_w2, gate_w):
        SK = A_k_cache.shape[2]
        W = min(4096, max(256, SK // 4))
        kt = jnp.transpose(A_k_cache, (0, 1, 3, 2))
        vt = jnp.transpose(A_v_cache, (0, 1, 3, 2))
        anyspec = pl.BlockSpec(memory_space=pl.ANY)
        NC = W // CW
        return pl.pallas_call(
            functools.partial(_kernel, SK=SK, W=W, WQ=WQ, W13=W13, G=G, SPLIT=SPLIT, WOPOS=WOPOS),
            out_shape=jax.ShapeDtypeStruct((1, 1, D), bf16),
            in_specs=[anyspec] * 9,
            out_specs=pl.BlockSpec(memory_space=pltpu.VMEM),
            scratch_shapes=[
                pltpu.VMEM((1, D), bf16), pltpu.VMEM((D,), bf16),
                pltpu.VMEM((D, H * DH), bf16), pltpu.VMEM((2, DH, D), bf16),
                pltpu.VMEM((D, F), bf16), pltpu.VMEM((D, F), bf16), pltpu.VMEM((F, D), bf16),
                pltpu.VMEM((2, DH, W), bf16), pltpu.VMEM((2, DH, W), bf16),
                pltpu.VMEM((H, M, DH), bf16), pltpu.VMEM((2, M, W), f32),
                pltpu.VMEM((M, F), bf16), pltpu.VMEM((M, D), f32),
                pltpu.SemaphoreType.DMA((2 * NC,)), pltpu.SemaphoreType.DMA((D // 128,)), pltpu.SemaphoreType.DMA((2,)),
            ],
            compiler_params=pltpu.CompilerParams(vmem_limit_bytes=100 * 2**20, disable_semaphore_checks=True, disable_bounds_checks=True, **cp),
        )(A_x, kt, vt, A_wq, A_wo, B_w1, B_w3, B_w2, gate_w)
    return kernel

_impl = _make()


@jax.jit
def pallas_gated_mix__sliding_block_cached__glu_gated_swiglu__decode_kernel(
    A_x, A_k_cache, A_v_cache, A_wq, A_wo, B_x, B_w1, B_w3, B_w2, gate_w
):
    return _impl(A_x, A_k_cache, A_v_cache, A_wq, A_wo, B_x, B_w1, B_w3, B_w2, gate_w)
```

```python
import functools

import jax
import jax.numpy as jnp
import jax.experimental.pallas as pl
import jax.experimental.pallas.tpu as pltpu

H, DH = 32, 192
M = 8
CW = 128
G = 4
W_ROWS, W_COLS = 64, 384
WO_ROWS = 32
K_PAD = 2 * CW


def _kernel(x_hbm, k_hbm, v_hbm, wq_hbm, wo_hbm, w1_hbm, w3_hbm, w2_hbm, gw_hbm, o_ref,
            x_v, gw_v, wq_v, wo_v, w1_v, w3_v, w2_v, kbuf, vbuf, q_scr, s_scr, p_scr, h_scr, b_scr,
            sems, sem_o, sem_s, *, SK, W, D, F):
    f32, bf16 = jnp.float32, jnp.bfloat16
    NC = W // CW
    NO = DH // WO_ROWS
    R = 2 * NC
    GW = G * CW
    scale = DH ** -0.5
    nt = (((1,), (1,)), ((), ()))

    def par(h):
        return h % 2 if isinstance(h, int) else h & 1

    def k_copy(h, c, sem=None):
        return pltpu.make_async_copy(k_hbm.at[0, h, :, pl.ds(SK - W + c * CW, CW)],
                                     kbuf.at[par(h), :, pl.ds(c * CW, CW)],
                                     sems.at[2 * c] if sem is None else sem)

    def v_copy(h, c):
        return pltpu.make_async_copy(v_hbm.at[0, h, :, pl.ds(SK - W + c * CW, CW)],
                                     vbuf.at[par(h), :, pl.ds(c * CW, CW)], sems.at[2 * c + 1])

    def o_copy(h, i):
        r = h * DH + i * WO_ROWS
        if not isinstance(r, int):
            r = pl.multiple_of(r, WO_ROWS)
        return pltpu.make_async_copy(wo_hbm.at[pl.ds(r, WO_ROWS), :],
                                     wo_v.at[par(h), pl.ds(i * WO_ROWS, WO_ROWS), :], sem_o.at[i])

    def w_copy(src, dst, r0, nr, c0, ncol):
        return lambda sem: pltpu.make_async_copy(src.at[pl.ds(r0, nr), pl.ds(c0, ncol)],
                                                 dst.at[pl.ds(r0, nr), pl.ds(c0, ncol)], sem)

    def qk(h1, c0, n, m_run):
        s = jnp.dot(q_scr[h1], kbuf[par(h1), :, pl.ds(c0, n)], preferred_element_type=f32) * scale
        s_scr[par(h1), :, pl.ds(c0, n)] = s
        for t in range(n // CW):
            m_run = jnp.maximum(m_run, s[:, t * CW:(t + 1) * CW])
        return m_run

    def pv(h, c0, n, m, l_vec, o_acc):
        p = jnp.exp(s_scr[par(h), :, pl.ds(c0, n)] - m)
        for t in range(n // CW):
            l_vec = l_vec + p[:, t * CW:(t + 1) * CW]
        o_acc = o_acc + jax.lax.dot_general(p.astype(bf16), vbuf[par(h), :, pl.ds(c0, n)], nt,
                                            preferred_element_type=f32)
        return l_vec, o_acc

    blocks = []
    for c0 in range(0, F, W_COLS):
        for name, src, dst in (('g', w1_hbm, w1_v), ('u', w3_hbm, w3_v)):
            blocks.append((name, c0, W_COLS,
                           [w_copy(src, dst, r0, W_ROWS, c0, W_COLS) for r0 in range(0, D, W_ROWS)]))
    for c0 in range(0, D, 128):
        blocks.append(('b', c0, 128, [w_copy(w2_hbm, w2_v, r0, DH, c0, 128) for r0 in range(0, F, DH)]))
    for c0 in range(0, H * DH, W_COLS):
        blocks.append(('q', c0, W_COLS,
                       [w_copy(wq_hbm, wq_v, r0, W_ROWS, c0, W_COLS) for r0 in range(0, D, W_ROWS)]))
    for gi in range(NC // G):
        blocks.append(('k', gi * GW, GW, [functools.partial(k_copy, 0, gi * G + t) for t in range(G)]))
    pro = [cp for b in blocks for cp in b[3]]
    P = len(pro)

    def stream_copy(j):
        if j < P:
            return pro[j](sems.at[(j - P) % R])
        i = j - P
        return k_copy(1, i // 2) if i % 2 == 0 else v_copy(0, i // 2)

    def stream_start(j):
        stream_copy(j).start(priority=(j - P) % 2)

    x_copy = pltpu.make_async_copy(x_hbm.at[0], x_v, sem_s.at[0])
    gw_copy = pltpu.make_async_copy(gw_hbm, gw_v, sem_s.at[1])
    x_copy.start()
    gw_copy.start()
    for j in range(R):
        stream_start(j)

    j = 0
    xb = g = gate = None
    m_vec = jnp.full((M, CW), -jnp.inf, f32)
    for name, c0, ncol, copies in blocks:
        for _ in copies:
            stream_copy(j).wait()
            stream_start(j + R)
            if j >= P - NO:
                o_copy(0, j - (P - NO)).start(priority=j % 2)
            j += 1
        if xb is None:
            x_copy.wait()
            gw_copy.wait()
            xb = jnp.broadcast_to(x_v[...], (M, D))
            xg = x_v[...].astype(f32) * gw_v[...].astype(f32).reshape(1, D)
            g = jax.nn.sigmoid(jnp.sum(xg, axis=-1, keepdims=True))
        if name == 'k':
            m_vec = qk(0, c0, ncol, m_vec)
        elif name == 'b':
            b_scr[:, pl.ds(c0, ncol)] = jnp.dot(h_scr[...], w2_v[:, pl.ds(c0, ncol)],
                                                preferred_element_type=f32)
        else:
            w_v = {'q': wq_v, 'g': w1_v, 'u': w3_v}[name]
            d = jnp.dot(xb, w_v[:, pl.ds(c0, ncol)], preferred_element_type=f32)
            if name == 'q':
                qb = d.astype(bf16)
                for t in range(ncol // DH):
                    q_scr[c0 // DH + t] = qb[:, t * DH:(t + 1) * DH]
            elif name == 'g':
                gate = d
            else:
                h_scr[:, pl.ds(c0, ncol)] = (gate * jax.nn.sigmoid(gate) * d).astype(bf16)

    def iteration(h, m_vec, out_acc, last_k):
        m = jnp.max(m_vec, axis=-1, keepdims=True)
        l_vec = jnp.zeros((M, CW), f32)
        o_acc = jnp.zeros((M, DH), f32)
        m_new = jnp.full((M, CW), -jnp.inf, f32)
        for gi in range(NC // G):
            for t in range(G):
                c = gi * G + t
                k_copy(h + 1, c).wait()
                if not last_k:
                    k_copy(h + 2, c).start(priority=0)
                v_copy(h, c).wait()
                if not last_k:
                    v_copy(h + 1, c).start(priority=1)
                else:
                    v_copy(h + 1, c // 2 + (c % 2) * (NC // 2)).start(priority=c % 2)
            if gi == NC // G - 1:
                for i in range(NO):
                    o_copy(h, i).wait()
                    o_copy(h + 1, i).start(priority=1 if last_k else i % 2)
            m_new = qk(h + 1, gi * GW, GW, m_new)
            l_vec, o_acc = pv(h, gi * GW, GW, m, l_vec, o_acc)
        l = jnp.sum(l_vec, axis=-1, keepdims=True)
        o = (o_acc / l).astype(bf16)
        out_acc = out_acc + jnp.dot(o, wo_v[par(h)], preferred_element_type=f32)
        return m_new, out_acc

    out_acc = jnp.zeros((M, D), f32)
    m_vec, out_acc = jax.lax.fori_loop(
        0, H - 2, lambda h, carry: iteration(h, carry[0], carry[1], False), (m_vec, out_acc))
    m_vec, out_acc = iteration(H - 2, m_vec, out_acc, True)

    h = H - 1
    m = jnp.max(m_vec, axis=-1, keepdims=True)
    p = jnp.exp(s_scr[par(h)] - m)
    l = jnp.sum(p, axis=-1, keepdims=True)
    p_scr[...] = p.astype(bf16)
    rl = 1.0 / l
    o_acc = jnp.zeros((M, DH), f32)
    c0 = 0
    for n in (NC // 2, NC // 4, NC // 8, NC // 8):
        for c in range(c0, c0 + n):
            v_copy(h, c).wait()
        o_acc = o_acc + jax.lax.dot_general(p_scr[:, pl.ds(c0 * CW, n * CW)],
                                            vbuf[par(h), :, pl.ds(c0 * CW, n * CW)], nt,
                                            preferred_element_type=f32)
        c0 += n
    o = (o_acc * rl).astype(bf16)
    pre = g * out_acc[0:1] + (1 - g) * b_scr[0:1, :]
    for i in range(NO):
        o_copy(h, i).wait()
    a = jnp.dot(o, wo_v[par(h)], preferred_element_type=f32)
    o_ref[0] = (pre + g * a[0:1]).astype(o_ref.dtype)


@jax.jit
def pallas_gated_mix__sliding_block_cached__glu_gated_swiglu__decode_kernel(
    A_x: jax.Array,
    A_k_cache: jax.Array,
    A_v_cache: jax.Array,
    A_wq: jax.Array,
    A_wo: jax.Array,
    B_x: jax.Array,
    B_w1: jax.Array,
    B_w3: jax.Array,
    B_w2: jax.Array,
    gate_w: jax.Array,
):
    del B_x
    D = A_x.shape[-1]
    F = B_w1.shape[-1]
    SK = A_k_cache.shape[2]
    W = min(4096, max(256, SK // 4))
    NC = W // CW
    assert A_k_cache.shape == (1, H, SK, DH) and A_x.shape == (1, 1, D)
    assert NC % 8 == 0 and NC % G == 0 and F % W_COLS == 0 and F % DH == 0 and D % 128 == 0

    kt = jnp.transpose(A_k_cache, (0, 1, 3, 2))
    vt = jnp.transpose(A_v_cache, (0, 1, 3, 2))

    f32, bf16 = jnp.float32, jnp.bfloat16
    return pl.pallas_call(
        functools.partial(_kernel, SK=SK, W=W, D=D, F=F),
        out_shape=jax.ShapeDtypeStruct((1, 1, D), A_x.dtype),
        in_specs=[pl.BlockSpec(memory_space=pl.ANY)] * 9,
        out_specs=pl.BlockSpec(memory_space=pltpu.VMEM),
        scratch_shapes=[
            pltpu.VMEM((1, D), bf16),
            pltpu.VMEM((D,), bf16),
            pltpu.VMEM((D, H * DH), bf16),
            pltpu.VMEM((2, DH, D), bf16),
            pltpu.VMEM((D, F), bf16),
            pltpu.VMEM((D, F), bf16),
            pltpu.VMEM((F, D), bf16),
            pltpu.VMEM((2, DH, W + K_PAD), bf16),
            pltpu.VMEM((2, DH, W), bf16),
            pltpu.VMEM((H, M, DH), bf16),
            pltpu.VMEM((2, M, W), f32),
            pltpu.VMEM((M, W), bf16),
            pltpu.VMEM((M, F), bf16),
            pltpu.VMEM((M, D), f32),
            pltpu.SemaphoreType.DMA((2 * NC,)),
            pltpu.SemaphoreType.DMA((DH // WO_ROWS,)),
            pltpu.SemaphoreType.DMA((2,)),
        ],
        compiler_params=pltpu.CompilerParams(
            vmem_limit_bytes=100 * 2**20,
            disable_bounds_checks=True,
            disable_semaphore_checks=True,
        ),
    )(A_x, kt, vt, A_wq, A_wo, B_w1, B_w3, B_w2, gate_w)
```

```python
import functools

import jax
import jax.numpy as jnp
import jax.experimental.pallas as pl
import jax.experimental.pallas.tpu as pltpu

H, DH = 32, 192
M = 8
CW = 128
G = 4
W_ROWS, W_COLS = 64, 384
WO_ROWS = 32
K_PAD = 2 * CW


def _kernel(x_hbm, k_hbm, v_hbm, wq_hbm, wo_hbm, w1_hbm, w3_hbm, w2_hbm, gw_hbm, o_ref,
            x_v, gw_v, wq_v, wo_v, w1_v, w3_v, w2_v, kbuf, vbuf, q_scr, s_scr, p_scr, h_scr, b_scr,
            sems, sem_o, sem_s, *, SK, W, D, F):
    f32, bf16 = jnp.float32, jnp.bfloat16
    NC = W // CW
    NO = DH // WO_ROWS
    R = 2 * NC
    GW = G * CW
    scale = DH ** -0.5
    nt = (((1,), (1,)), ((), ()))

    def par(h):
        return h % 2 if isinstance(h, int) else h & 1

    def k_copy(h, c, sem=None):
        return pltpu.make_async_copy(k_hbm.at[0, h, :, pl.ds(SK - W + c * CW, CW)],
                                     kbuf.at[par(h), :, pl.ds(c * CW, CW)],
                                     sems.at[2 * c] if sem is None else sem)

    def v_copy(h, c):
        return pltpu.make_async_copy(v_hbm.at[0, h, :, pl.ds(SK - W + c * CW, CW)],
                                     vbuf.at[par(h), :, pl.ds(c * CW, CW)], sems.at[2 * c + 1])

    def last_v_order(c):
        return c // 2 + (c % 2) * (NC // 2)

    def last_v_copy(c):
        cv = last_v_order(c)
        return pltpu.make_async_copy(v_hbm.at[0, H - 1, :, pl.ds(SK - W + cv * CW, CW)],
                                     vbuf.at[par(H - 1), :, pl.ds(cv * CW, CW)], sems.at[2 * c])

    def o_copy(h, i):
        r = h * DH + i * WO_ROWS
        if not isinstance(r, int):
            r = pl.multiple_of(r, WO_ROWS)
        return pltpu.make_async_copy(wo_hbm.at[pl.ds(r, WO_ROWS), :],
                                     wo_v.at[par(h), pl.ds(i * WO_ROWS, WO_ROWS), :], sem_o.at[i])

    def w_copy(src, dst, r0, nr, c0, ncol):
        return lambda sem: pltpu.make_async_copy(src.at[pl.ds(r0, nr), pl.ds(c0, ncol)],
                                                 dst.at[pl.ds(r0, nr), pl.ds(c0, ncol)], sem)

    def qk(h1, c0, n, m_run):
        s = jnp.dot(q_scr[h1], kbuf[par(h1), :, pl.ds(c0, n)], preferred_element_type=f32) * scale
        s_scr[par(h1), :, pl.ds(c0, n)] = s
        for t in range(n // CW):
            m_run = jnp.maximum(m_run, s[:, t * CW:(t + 1) * CW])
        return m_run

    def pv(h, c0, n, m, l_vec, o_acc):
        p = jnp.exp(s_scr[par(h), :, pl.ds(c0, n)] - m)
        for t in range(n // CW):
            l_vec = l_vec + p[:, t * CW:(t + 1) * CW]
        o_acc = o_acc + jax.lax.dot_general(p.astype(bf16), vbuf[par(h), :, pl.ds(c0, n)], nt,
                                            preferred_element_type=f32)
        return l_vec, o_acc

    blocks = []
    for c0 in range(0, F, W_COLS):
        for name, src, dst in (('g', w1_hbm, w1_v), ('u', w3_hbm, w3_v)):
            blocks.append((name, c0, W_COLS,
                           [w_copy(src, dst, r0, W_ROWS, c0, W_COLS) for r0 in range(0, D, W_ROWS)]))
    for c0 in range(0, D, 128):
        blocks.append(('b', c0, 128, [w_copy(w2_hbm, w2_v, r0, DH, c0, 128) for r0 in range(0, F, DH)]))
    for c0 in range(0, H * DH, W_COLS):
        blocks.append(('q', c0, W_COLS,
                       [w_copy(wq_hbm, wq_v, r0, W_ROWS, c0, W_COLS) for r0 in range(0, D, W_ROWS)]))
    for gi in range(NC // G):
        blocks.append(('k', gi * GW, GW, [functools.partial(k_copy, 0, gi * G + t) for t in range(G)]))
    pro = [cp for b in blocks for cp in b[3]]
    P = len(pro)

    def stream_copy(j):
        if j < P:
            return pro[j](sems.at[(j - P) % R])
        i = j - P
        return k_copy(1, i // 2) if i % 2 == 0 else v_copy(0, i // 2)

    def stream_start(j):
        stream_copy(j).start(priority=(j - P) % 2)

    x_copy = pltpu.make_async_copy(x_hbm.at[0], x_v, sem_s.at[0])
    gw_copy = pltpu.make_async_copy(gw_hbm, gw_v, sem_s.at[1])
    x_copy.start()
    gw_copy.start()
    for j in range(R):
        stream_start(j)

    j = 0
    xb = g = gate = None
    m_vec = jnp.full((M, CW), -jnp.inf, f32)
    for name, c0, ncol, copies in blocks:
        for _ in copies:
            stream_copy(j).wait()
            stream_start(j + R)
            if j >= P - NO:
                o_copy(0, j - (P - NO)).start(priority=j % 2)
            j += 1
        if xb is None:
            x_copy.wait()
            gw_copy.wait()
            xb = jnp.broadcast_to(x_v[...], (M, D))
            xg = x_v[...].astype(f32) * gw_v[...].astype(f32).reshape(1, D)
            g = jax.nn.sigmoid(jnp.sum(xg, axis=-1, keepdims=True))
        if name == 'k':
            m_vec = qk(0, c0, ncol, m_vec)
        elif name == 'b':
            b_scr[:, pl.ds(c0, ncol)] = jnp.dot(h_scr[...], w2_v[:, pl.ds(c0, ncol)],
                                                preferred_element_type=f32)
        else:
            w_v = {'q': wq_v, 'g': w1_v, 'u': w3_v}[name]
            d = jnp.dot(xb, w_v[:, pl.ds(c0, ncol)], preferred_element_type=f32)
            if name == 'q':
                qb = d.astype(bf16)
                for t in range(ncol // DH):
                    q_scr[c0 // DH + t] = qb[:, t * DH:(t + 1) * DH]
            elif name == 'g':
                gate = d
            else:
                h_scr[:, pl.ds(c0, ncol)] = (gate * jax.nn.sigmoid(gate) * d).astype(bf16)

    def iteration(h, m_vec, out_acc, last_k):
        m = jnp.max(m_vec, axis=-1, keepdims=True)
        l_vec = jnp.zeros((M, CW), f32)
        o_acc = jnp.zeros((M, DH), f32)
        m_new = jnp.full((M, CW), -jnp.inf, f32)
        for gi in range(NC // G):
            for t in range(G):
                c = gi * G + t
                k_copy(h + 1, c).wait()
                if not last_k:
                    k_copy(h + 2, c).start(priority=0)
                v_copy(h, c).wait()
                if not last_k:
                    v_copy(h + 1, c).start(priority=1)
                else:
                    last_v_copy(c).start(priority=c % 2)
            if gi == NC // G - 1:
                for i in range(NO):
                    o_copy(h, i).wait()
                    o_copy(h + 1, i).start(priority=1 if last_k else i % 2)
            m_new = qk(h + 1, gi * GW, GW, m_new)
            l_vec, o_acc = pv(h, gi * GW, GW, m, l_vec, o_acc)
        l = jnp.sum(l_vec, axis=-1, keepdims=True)
        o = (o_acc / l).astype(bf16)
        out_acc = out_acc + jnp.dot(o, wo_v[par(h)], preferred_element_type=f32)
        return m_new, out_acc

    out_acc = jnp.zeros((M, D), f32)
    m_vec, out_acc = jax.lax.fori_loop(
        0, H - 2, lambda h, carry: iteration(h, carry[0], carry[1], False), (m_vec, out_acc))
    m_vec, out_acc = iteration(H - 2, m_vec, out_acc, True)

    h = H - 1
    m = jnp.max(m_vec, axis=-1, keepdims=True)
    p = jnp.exp(s_scr[par(h)] - m)
    l = jnp.sum(p, axis=-1, keepdims=True)
    p_scr[...] = p.astype(bf16)
    rl = 1.0 / l
    o_acc = jnp.zeros((M, DH), f32)
    step_of = {last_v_order(c): c for c in range(NC)}
    c0 = 0
    for n in (NC // 2, NC // 4, NC // 8, NC // 8):
        for cv in range(c0, c0 + n):
            last_v_copy(step_of[cv]).wait()
        o_acc = o_acc + jax.lax.dot_general(p_scr[:, pl.ds(c0 * CW, n * CW)],
                                            vbuf[par(h), :, pl.ds(c0 * CW, n * CW)], nt,
                                            preferred_element_type=f32)
        c0 += n
    o = (o_acc * rl).astype(bf16)
    pre = g * out_acc[0:1] + (1 - g) * b_scr[0:1, :]
    for i in range(NO):
        o_copy(h, i).wait()
    a = jnp.dot(o, wo_v[par(h)], preferred_element_type=f32)
    o_ref[0] = (pre + g * a[0:1]).astype(o_ref.dtype)


@jax.jit
def pallas_gated_mix__sliding_block_cached__glu_gated_swiglu__decode_kernel(
    A_x: jax.Array,
    A_k_cache: jax.Array,
    A_v_cache: jax.Array,
    A_wq: jax.Array,
    A_wo: jax.Array,
    B_x: jax.Array,
    B_w1: jax.Array,
    B_w3: jax.Array,
    B_w2: jax.Array,
    gate_w: jax.Array,
):
    del B_x
    D = A_x.shape[-1]
    F = B_w1.shape[-1]
    SK = A_k_cache.shape[2]
    W = min(4096, max(256, SK // 4))
    NC = W // CW
    assert A_k_cache.shape == (1, H, SK, DH) and A_x.shape == (1, 1, D)
    assert NC % 8 == 0 and NC % G == 0 and F % W_COLS == 0 and F % DH == 0 and D % 128 == 0

    kt = jnp.transpose(A_k_cache, (0, 1, 3, 2))
    vt = jnp.transpose(A_v_cache, (0, 1, 3, 2))

    f32, bf16 = jnp.float32, jnp.bfloat16
    return pl.pallas_call(
        functools.partial(_kernel, SK=SK, W=W, D=D, F=F),
        out_shape=jax.ShapeDtypeStruct((1, 1, D), A_x.dtype),
        in_specs=[pl.BlockSpec(memory_space=pl.ANY)] * 9,
        out_specs=pl.BlockSpec(memory_space=pltpu.VMEM),
        scratch_shapes=[
            pltpu.VMEM((1, D), bf16),
            pltpu.VMEM((D,), bf16),
            pltpu.VMEM((D, H * DH), bf16),
            pltpu.VMEM((2, DH, D), bf16),
            pltpu.VMEM((D, F), bf16),
            pltpu.VMEM((D, F), bf16),
            pltpu.VMEM((F, D), bf16),
            pltpu.VMEM((2, DH, W + K_PAD), bf16),
            pltpu.VMEM((2, DH, W), bf16),
            pltpu.VMEM((H, M, DH), bf16),
            pltpu.VMEM((2, M, W), f32),
            pltpu.VMEM((M, W), bf16),
            pltpu.VMEM((M, F), bf16),
            pltpu.VMEM((M, D), f32),
            pltpu.SemaphoreType.DMA((2 * NC,)),
            pltpu.SemaphoreType.DMA((DH // WO_ROWS,)),
            pltpu.SemaphoreType.DMA((2,)),
        ],
        compiler_params=pltpu.CompilerParams(
            vmem_limit_bytes=100 * 2**20,
            disable_bounds_checks=True,
            disable_semaphore_checks=True,
        ),
    )(A_x, kt, vt, A_wq, A_wo, B_w1, B_w3, B_w2, gate_w)
```

```python
import functools

import jax
import jax.numpy as jnp
import jax.experimental.pallas as pl
import jax.experimental.pallas.tpu as pltpu

H, DH = 32, 192
M = 8
CW = 128
G = 4
W_BLOCK = 384
W_ROWS, W_COLS = 160, 128
W2_ROWS = 32
WO_ROWS = 32
K_PAD = 2 * CW


def _kernel(x_hbm, k_hbm, v_hbm, wq_hbm, wo_hbm, w1_hbm, w3_hbm, w2_hbm, gw_hbm, o_ref,
            x_v, gw_v, wq_v, wo_v, w1_v, w3_v, w2_v, kbuf, vbuf, q_scr, s_scr, p_scr, h_scr, b_scr,
            sems, sem_o, sem_s, *, SK, W, D, F):
    f32, bf16 = jnp.float32, jnp.bfloat16
    NC = W // CW
    NO = DH // WO_ROWS
    R = 2 * NC
    GW = G * CW
    scale = DH ** -0.5
    nt = (((1,), (1,)), ((), ()))

    def par(h):
        return h % 2 if isinstance(h, int) else h & 1

    def k_copy(h, c, sem=None):
        return pltpu.make_async_copy(k_hbm.at[0, h, :, pl.ds(SK - W + c * CW, CW)],
                                     kbuf.at[par(h), :, pl.ds(c * CW, CW)],
                                     sems.at[2 * c] if sem is None else sem)

    def v_copy(h, c):
        return pltpu.make_async_copy(v_hbm.at[0, h, :, pl.ds(SK - W + c * CW, CW)],
                                     vbuf.at[par(h), :, pl.ds(c * CW, CW)], sems.at[2 * c + 1])

    def last_v_order(c):
        return c // 2 + (c % 2) * (NC // 2)

    def last_v_copy(c):
        cv = last_v_order(c)
        return pltpu.make_async_copy(v_hbm.at[0, H - 1, :, pl.ds(SK - W + cv * CW, CW)],
                                     vbuf.at[par(H - 1), :, pl.ds(cv * CW, CW)], sems.at[2 * c])

    def o_copy(h, i):
        r = h * DH + i * WO_ROWS
        if not isinstance(r, int):
            r = pl.multiple_of(r, WO_ROWS)
        return pltpu.make_async_copy(wo_hbm.at[pl.ds(r, WO_ROWS), :],
                                     wo_v.at[par(h), pl.ds(i * WO_ROWS, WO_ROWS), :], sem_o.at[i])

    def w_copy(src, dst, r0, nr, c0, ncol):
        return lambda sem: pltpu.make_async_copy(src.at[pl.ds(r0, nr), pl.ds(c0, ncol)],
                                                 dst.at[pl.ds(r0, nr), pl.ds(c0, ncol)], sem)

    def qk(h1, c0, n, m_run):
        s = jnp.dot(q_scr[h1], kbuf[par(h1), :, pl.ds(c0, n)], preferred_element_type=f32) * scale
        s_scr[par(h1), :, pl.ds(c0, n)] = s
        for t in range(n // CW):
            m_run = jnp.maximum(m_run, s[:, t * CW:(t + 1) * CW])
        return m_run

    def pv(h, c0, n, m, l_vec, o_acc):
        p = jnp.exp(s_scr[par(h), :, pl.ds(c0, n)] - m)
        for t in range(n // CW):
            l_vec = l_vec + p[:, t * CW:(t + 1) * CW]
        o_acc = o_acc + jax.lax.dot_general(p.astype(bf16), vbuf[par(h), :, pl.ds(c0, n)], nt,
                                            preferred_element_type=f32)
        return l_vec, o_acc

    blocks = []
    def w_block(name, src, dst, c0):
        return (name, c0, W_BLOCK, [w_copy(src, dst, r0, W_ROWS, c1, W_COLS)
                                    for c1 in range(c0, c0 + W_BLOCK, W_COLS) for r0 in range(0, D, W_ROWS)])

    for c0 in range(0, H * DH, W_BLOCK):
        blocks.append(w_block('q', wq_hbm, wq_v, c0))
    for gi in range(NC // G):
        blocks.append(('k', gi * GW, GW, [functools.partial(k_copy, 0, gi * G + t) for t in range(G)]))
    for c0 in range(0, F, W_BLOCK):
        blocks.append(w_block('g', w1_hbm, w1_v, c0))
        blocks.append(w_block('u', w3_hbm, w3_v, c0))
    blocks.append(('b', 0, D, [w_copy(w2_hbm, w2_v, r0, W2_ROWS, 0, D) for r0 in range(0, F, W2_ROWS)]))
    pro = [cp for b in blocks for cp in b[3]]
    P = len(pro)

    def stream_copy(j):
        if j < P:
            return pro[j](sems.at[(j - P) % R])
        i = j - P
        return k_copy(1, i // 2) if i % 2 == 0 else v_copy(0, i // 2)

    def stream_start(j):
        stream_copy(j).start(priority=(j - P) % 2)

    x_copy = pltpu.make_async_copy(x_hbm.at[0], x_v, sem_s.at[0])
    gw_copy = pltpu.make_async_copy(gw_hbm, gw_v, sem_s.at[1])
    x_copy.start()
    gw_copy.start()
    for j in range(R):
        stream_start(j)

    j = 0
    xb = g = gate = None
    m_vec = jnp.full((M, CW), -jnp.inf, f32)
    for name, c0, ncol, copies in blocks:
        for _ in copies:
            stream_copy(j).wait()
            stream_start(j + R)
            if j >= P - NO:
                o_copy(0, j - (P - NO)).start(priority=j % 2)
            j += 1
        if xb is None:
            x_copy.wait()
            gw_copy.wait()
            xb = jnp.broadcast_to(x_v[...], (M, D))
            xg = x_v[...].astype(f32) * gw_v[...].astype(f32).reshape(1, D)
            g = jax.nn.sigmoid(jnp.sum(xg, axis=-1, keepdims=True))
        if name == 'k':
            m_vec = qk(0, c0, ncol, m_vec)
        elif name == 'b':
            b_scr[:, pl.ds(c0, ncol)] = jnp.dot(h_scr[...], w2_v[:, pl.ds(c0, ncol)],
                                                preferred_element_type=f32)
        else:
            w_v = {'q': wq_v, 'g': w1_v, 'u': w3_v}[name]
            d = jnp.dot(xb, w_v[:, pl.ds(c0, ncol)], preferred_element_type=f32)
            if name == 'q':
                qb = d.astype(bf16)
                for t in range(ncol // DH):
                    q_scr[c0 // DH + t] = qb[:, t * DH:(t + 1) * DH]
            elif name == 'g':
                gate = d
            else:
                h_scr[:, pl.ds(c0, ncol)] = (gate * jax.nn.sigmoid(gate) * d).astype(bf16)

    def iteration(h, m_vec, out_acc, last_k):
        m = jnp.max(m_vec, axis=-1, keepdims=True)
        l_vec = jnp.zeros((M, CW), f32)
        o_acc = jnp.zeros((M, DH), f32)
        m_new = jnp.full((M, CW), -jnp.inf, f32)
        NG = NC // G
        for gi in range(NG):
            for t in range(G):
                k_copy(h + 1, gi * G + t).wait()
            for t in range(G):
                c = gi * G + t
                if not last_k:
                    k_copy(h + 2, c).start(priority=0)
                v_copy(h, c).wait()
                if not last_k:
                    v_copy(h + 1, c).start(priority=1)
                else:
                    last_v_copy(c).start(priority=c % 2)
                if t == 0:
                    m_new = qk(h + 1, gi * GW, GW, m_new)
                if t == G // 2 and gi > 0:
                    l_vec, o_acc = pv(h, (gi - 1) * GW, GW, m, l_vec, o_acc)
        for i in range(NO):
            o_copy(h, i).wait()
            o_copy(h + 1, i).start(priority=1 if last_k else i % 2)
        l_vec, o_acc = pv(h, (NG - 1) * GW, GW, m, l_vec, o_acc)
        l = jnp.sum(l_vec, axis=-1, keepdims=True)
        o = (o_acc / l).astype(bf16)
        out_acc = out_acc + jnp.dot(o, wo_v[par(h)], preferred_element_type=f32)
        return m_new, out_acc

    out_acc = jnp.zeros((M, D), f32)
    m_vec, out_acc = jax.lax.fori_loop(
        0, H - 2, lambda h, carry: iteration(h, carry[0], carry[1], False), (m_vec, out_acc))
    m_vec, out_acc = iteration(H - 2, m_vec, out_acc, True)

    h = H - 1
    m = jnp.max(m_vec, axis=-1, keepdims=True)
    p = jnp.exp(s_scr[par(h)] - m)
    l = jnp.sum(p, axis=-1, keepdims=True)
    p_scr[...] = p.astype(bf16)
    rl = 1.0 / l
    o_acc = jnp.zeros((M, DH), f32)
    step_of = {last_v_order(c): c for c in range(NC)}
    c0 = 0
    for n in (3 * NC // 8, 3 * NC // 8, NC // 4):
        for cv in range(c0, c0 + n):
            last_v_copy(step_of[cv]).wait()
        o_acc = o_acc + jax.lax.dot_general(p_scr[:, pl.ds(c0 * CW, n * CW)],
                                            vbuf[par(h), :, pl.ds(c0 * CW, n * CW)], nt,
                                            preferred_element_type=f32)
        c0 += n
    o = (o_acc * rl).astype(bf16)
    pre = g * out_acc[0:1] + (1 - g) * b_scr[0:1, :]
    for i in range(NO):
        o_copy(h, i).wait()
    a = jnp.dot(o, wo_v[par(h)], preferred_element_type=f32)
    o_ref[0] = (pre + g * a[0:1]).astype(o_ref.dtype)


@jax.jit
def pallas_gated_mix__sliding_block_cached__glu_gated_swiglu__decode_kernel(
    A_x: jax.Array,
    A_k_cache: jax.Array,
    A_v_cache: jax.Array,
    A_wq: jax.Array,
    A_wo: jax.Array,
    B_x: jax.Array,
    B_w1: jax.Array,
    B_w3: jax.Array,
    B_w2: jax.Array,
    gate_w: jax.Array,
):
    del B_x
    D = A_x.shape[-1]
    F = B_w1.shape[-1]
    SK = A_k_cache.shape[2]
    W = min(4096, max(256, SK // 4))
    NC = W // CW
    assert A_k_cache.shape == (1, H, SK, DH) and A_x.shape == (1, 1, D)
    assert NC % 8 == 0 and NC % G == 0 and F % W_BLOCK == 0 and F % W2_ROWS == 0 and D % W_ROWS == 0

    kt = jnp.transpose(A_k_cache, (0, 1, 3, 2))
    vt = jnp.transpose(A_v_cache, (0, 1, 3, 2))

    f32, bf16 = jnp.float32, jnp.bfloat16
    return pl.pallas_call(
        functools.partial(_kernel, SK=SK, W=W, D=D, F=F),
        out_shape=jax.ShapeDtypeStruct((1, 1, D), A_x.dtype),
        in_specs=[pl.BlockSpec(memory_space=pl.ANY)] * 9,
        out_specs=pl.BlockSpec(memory_space=pltpu.VMEM),
        scratch_shapes=[
            pltpu.VMEM((1, D), bf16),
            pltpu.VMEM((D,), bf16),
            pltpu.VMEM((D, H * DH), bf16),
            pltpu.VMEM((2, DH, D), bf16),
            pltpu.VMEM((D, F), bf16),
            pltpu.VMEM((D, F), bf16),
            pltpu.VMEM((F, D), bf16),
            pltpu.VMEM((2, DH, W + K_PAD), bf16),
            pltpu.VMEM((2, DH, W), bf16),
            pltpu.VMEM((H, M, DH), bf16),
            pltpu.VMEM((2, M, W), f32),
            pltpu.VMEM((M, W), bf16),
            pltpu.VMEM((M, F), bf16),
            pltpu.VMEM((M, D), f32),
            pltpu.SemaphoreType.DMA((2 * NC,)),
            pltpu.SemaphoreType.DMA((DH // WO_ROWS,)),
            pltpu.SemaphoreType.DMA((2,)),
        ],
        compiler_params=pltpu.CompilerParams(
            vmem_limit_bytes=100 * 2**20,
            disable_semaphore_checks=True,
        ),
    )(A_x, kt, vt, A_wq, A_wo, B_w1, B_w3, B_w2, gate_w)
```
